```python
import jax
import jax.numpy as jnp

def _softmax(x, axis=-1):
    return jax.nn.softmax(x, axis=axis)

def _gelu(x):
    return jax.nn.gelu(x, approximate=True)

def _silu(x):
    return jax.nn.silu(x)

def _sigmoid(x):
    return jax.nn.sigmoid(x)

def _layernorm(x, axis=-1, eps=1e-05):
    m = jnp.mean(x, axis=axis, keepdims=True)
    v = jnp.var(x, axis=axis, keepdims=True)
    return (x - m) / jnp.sqrt(v + eps)

def _scatter_add(tgt, idx, src, axis=0):
    return tgt.at[idx].add(src)

def _segment_sum(src, seg, n):
    return jax.ops.segment_sum(src, seg, n)

class _Rng:

    def __init__(self, key):
        self._k = key

    def _next(self):
        self._k, sub = jax.random.split(self._k)
        return sub

    def normal(self, shape):
        return jax.random.normal(self._next(), shape, dtype=jnp.bfloat16)

    def randint(self, lo, hi, shape):
        return jax.random.randint(self._next(), shape, lo, hi, dtype=jnp.int32)

    def uniform(self, shape, lo=0.0, hi=1.0):
        return jax.random.uniform(self._next(), shape, jnp.bfloat16, lo, hi)

    def permutation(self, n):
        return jax.random.permutation(self._next(), n)
kernel_name = 'interleave_layers__linear_kernel_hedgehog__mixer_gmlp__prompt'

def _fwd_setup_inputs():
    _rng = _Rng(jax.random.key(int.from_bytes(__import__("os").urandom(4), "little")))
    _w = lambda a: (lambda t: t.astype(jnp.bfloat16) if jnp.issubdtype(t.dtype, jnp.floating) else t)(jnp.asarray(a))

    def _A_setup():
        B, S, D, H = (1, 2048, 640, 32)
        Dh = D // H
        return {'x': _w((lambda *s: _rng.normal(s) * 0.05)(B, S, D)), 'wqkv': _w((lambda *s: _rng.normal(s) * 0.05)(D, 3 * D)), 'w_phi': _w((lambda *s: _rng.normal(s) * 0.05)(H, Dh, Dh) * Dh ** (-0.5)), 'wo': _w((lambda *s: _rng.normal(s) * 0.05)(D, D))}
    _A_in = _A_setup()

    def _B_setup():
        B, S, D, F = (1, 2048, 640, 1536)
        Fh = F // 2
        return {'x': _w((lambda *s: _rng.normal(s) * 0.05)(B, S, D)), 'w_in': _w((lambda *s: _rng.normal(s) * 0.05)(D, 2 * Fh)), 'w_sp': _w(0.01 * (lambda *s: _rng.normal(s) * 0.05)(S, S)), 'b_sp': _w(1.0 + 0.01 * (lambda *s: _rng.normal(s) * 0.05)(S)), 'w_out': _w((lambda *s: _rng.normal(s) * 0.05)(Fh, D))}
    _B_in = _B_setup()
    return {'A_x': _A_in['x'], 'A_wqkv': _A_in['wqkv'], 'A_w_phi': _A_in['w_phi'], 'A_wo': _A_in['wo'], 'B_x': _B_in['x'], 'B_w_in': _B_in['w_in'], 'B_w_sp': _B_in['w_sp'], 'B_b_sp': _B_in['b_sp'], 'B_w_out': _B_in['w_out']}

def _fwd_reference(A_x, A_wqkv, A_w_phi, A_wo, B_x, B_w_in, B_w_sp, B_b_sp, B_w_out):

    def _A_ref(x, wqkv, w_phi, wo):
        B, S, D = x.shape
        H = 32
        Dh = D // H
        qkv = (lambda x, *d: x.transpose(*d))((x @ wqkv).reshape(B, S, 3, H, Dh), 2, 0, 3, 1, 4)
        q, k, v = (qkv[0], qkv[1], qkv[2])
        pq = jnp.einsum('bhsd,hdf->bhsf', q, w_phi)
        pk = jnp.einsum('bhsd,hdf->bhsf', k, w_phi)
        phi_q = jnp.concatenate([_softmax(pq, axis=-1), _softmax(-pq, axis=-1)], axis=-1)
        phi_k = jnp.concatenate([_softmax(pk, axis=-1), _softmax(-pk, axis=-1)], axis=-1)
        kv = jnp.einsum('bhsf,bhsd->bhfd', phi_k, v)
        z = jnp.einsum('bhsf->bhf', phi_k)
        num = jnp.einsum('bhqf,bhfd->bhqd', phi_q, kv)
        den = jnp.einsum('bhqf,bhf->bhq', phi_q, z)[..., None] + 1e-06
        o = num / den
        return (lambda x, *d: x.transpose(*d))(o, 0, 2, 1, 3).reshape(B, S, D) @ wo

    def _B_ref(x, w_in, w_sp, b_sp, w_out):
        B, S, D = x.shape
        F = w_in.shape[-1]
        Fh = F // 2
        z = _gelu(jnp.einsum('bsd,df->bsf', x, w_in))
        z1 = z[..., :Fh].copy()
        z2 = _layernorm(z[..., Fh:], axis=-1)
        g = jnp.einsum('ts,bsf->btf', w_sp, z2) + b_sp[None, :, None]
        return jnp.einsum('bsf,fd->bsd', z1 * g, w_out)
    x = A_x
    x = x + _A_ref(_layernorm(x, axis=-1), A_wqkv, A_w_phi, A_wo)
    x = x + _B_ref(_layernorm(x, axis=-1), B_w_in, B_w_sp, B_b_sp, B_w_out)
    x = x + _A_ref(_layernorm(x, axis=-1), A_wqkv, A_w_phi, A_wo)
    x = x + _B_ref(_layernorm(x, axis=-1), B_w_in, B_w_sp, B_b_sp, B_w_out)
    return x

def setup_inputs():
    _inp = _fwd_setup_inputs()
    _gk = jax.random.fold_in(jax.random.key(int.from_bytes(__import__("os").urandom(4), "little")), 2 ** 31 - 1)
    _shapes = [[1, 2048, 640]]
    _dtypes = ['bfloat16']
    _gks = jax.random.split(_gk, len(_shapes))
    _gs = [jax.random.normal(k, s, dtype=jnp.dtype(d)) * 0.05 for k, s, d in zip(_gks, _shapes, _dtypes)]
    _inp['grad_out'] = _gs[0]
    return _inp

def reference(A_x, A_wqkv, A_w_phi, A_wo, B_w_in, B_w_sp, B_b_sp, B_w_out, B_x, grad_out):
    _const = dict(B_x=B_x)

    def _f(*_d):
        return _fwd_reference(**{'A_x': _d[0], 'A_wqkv': _d[1], 'A_w_phi': _d[2], 'A_wo': _d[3], 'B_w_in': _d[4], 'B_w_sp': _d[5], 'B_b_sp': _d[6], 'B_w_out': _d[7], **_const})
    _out, _vjp = jax.vjp(_f, A_x, A_wqkv, A_w_phi, A_wo, B_w_in, B_w_sp, B_b_sp, B_w_out)
    _grads = _vjp(grad_out)
    _out0 = jnp.asarray(_out)
    return (_out0, *[jnp.asarray(_g) for _g in _grads])
```

```python
import jax
import jax.numpy as jnp
import jax.experimental.pallas as pl
import jax.experimental.pallas.tpu as pltpu

S = 2048
D = 640
DH = 20
NG = 8
GR = 80
FH = 768
F = 1536
C = 256
NC = S // C

A_H = 0
A_PQ = 640
A_PK = A_PQ + 1280
A_VA = A_PK + 1280
A_O = A_VA + 768
A_ROWS = A_O + 640
B_H = 0
B_GP = 640
B_Z1 = B_GP + 1536
B_G = B_Z1 + 768
B_ROWS = B_G + 768

F32 = jnp.float32
BF16 = jnp.bfloat16
_NT = (((1,), (1,)), ((), ()))
_TN = (((0,), (0,)), ((), ()))
_GC = 0.7978845608028654
_GK = 0.044715


def _dot(a, b):
    return jnp.dot(a, b, preferred_element_type=F32)


def _dot_nt(a, b):
    return jax.lax.dot_general(a, b, _NT, preferred_element_type=F32)


def _dot_tn(a, b):
    return jax.lax.dot_general(a, b, _TN, preferred_element_type=F32)


def _idiv(x, n):
    return jnp.floor((x.astype(F32) + 0.5) * (1.0 / n)).astype(jnp.int32)


def _ln(x):
    mu = jnp.mean(x, axis=0, keepdims=True)
    xc = x - mu
    var = jnp.mean(xc * xc, axis=0, keepdims=True)
    r = jax.lax.rsqrt(var + 1e-5)
    return xc * r, r


def _ln_bwd(dy, y, r):
    m1 = jnp.mean(dy, axis=0, keepdims=True)
    m2 = jnp.mean(dy * y, axis=0, keepdims=True)
    return r * (dy - m1 - y * m2)


def _g3(x):
    return x.reshape(10, 8, x.shape[-1])


def _g2(x):
    return x.reshape(GR, x.shape[-1])


def _red_sum(x3):
    y = jnp.sum(x3, axis=0)
    return y + pltpu.roll(y, 4, 0)


def _red_max(x3):
    y = jnp.max(x3, axis=0)
    return jnp.maximum(y, pltpu.roll(y, 4, 0))


def _red_min(x3):
    y = jnp.min(x3, axis=0)
    return jnp.minimum(y, pltpu.roll(y, 4, 0))


def _phi(p):
    p3 = _g3(p)
    ep = jnp.exp(p3 - _red_max(p3)[None])
    en = jnp.exp(_red_min(p3)[None] - p3)
    pp = ep * (1.0 / _red_sum(ep))[None]
    pn = en * (1.0 / _red_sum(en))[None]
    return _g2(pp), _g2(pn)


def _phi_bwd(pp, pn, dpp, dpn):
    pp3, pn3, dp3, dn3 = _g3(pp), _g3(pn), _g3(dpp), _g3(dpn)
    a = pp3 * (dp3 - _red_sum(pp3 * dp3)[None])
    b = pn3 * (dn3 - _red_sum(pn3 * dn3)[None])
    return _g2(a - b)


def _gelu_and_grad(a):
    a2 = a * a
    t = jnp.tanh(_GC * (a + _GK * a2 * a))
    hp = 0.5 * (1.0 + t)
    z = a * hp
    gp = hp + (0.5 * _GC) * a * (1.0 - t * t) * (1.0 + 3.0 * _GK * a2)
    return z, gp


def _kernel(
    x_hbm, wqkv_hbm, wphi_hbm, wo_hbm, win_hbm, wsp_hbm, bsp_hbm, wout_hbm, go_hbm,
    out_hbm, gx_hbm, dwqkv_hbm, dwphi_hbm, dwo_hbm, dwin_hbm, dwsp_hbm, db_hbm,
    dwout_hbm, stA_hbm, stB_hbm,
    x_v, go_v, wqkv_v, wphi_v, wo_v, win_v, wsp_v, bsp_v, wout_v,
    weT, we, woP, woPT, winT, woutT, bds_v, wqkvT,
    xs, actA, actB, z2_v, den_v, rA_v, rB_v, r2_v,
    kvacc, kv_v, kvT_v, dkv_v, dkvT_v,
    dg_v, dz1_v, dpq_v, work, dqkv_v,
    dwe_a, dwo_a, dwin_a, dwout_a, db_a, dwsp_v, dwphi_v, db_v,
    sem_in, sem_out, sem_st,
):
    def cslice(c):
        if isinstance(c, int):
            return pl.ds(c * C, C)
        return pl.ds(pl.multiple_of(c * C, C), C)

    in_pairs = [
        (x_hbm, x_v), (wqkv_hbm, wqkv_v), (wphi_hbm, wphi_v), (wo_hbm, wo_v),
        (win_hbm, win_v), (wout_hbm, wout_v), (bsp_hbm, bsp_v), (wsp_hbm, wsp_v),
        (go_hbm, go_v),
    ]
    in_cp = [pltpu.make_async_copy(s, d, sem_in.at[i]) for i, (s, d) in enumerate(in_pairs)]
    in_cp[1].start()
    in_cp[2].start()
    in_cp[0].start()

    def stash_out_A(c):
        return pltpu.make_async_copy(actA.at[c], stA_hbm.at[c], sem_st.at[0, c])

    def stash_out_B(c):
        return pltpu.make_async_copy(actB.at[c], stB_hbm.at[c], sem_st.at[1, c])

    def stash_in_A(c):
        return pltpu.make_async_copy(stA_hbm.at[c], actA.at[c], sem_st.at[2, c])

    def stash_in_B(c):
        return pltpu.make_async_copy(stB_hbm.at[c], actB.at[c], sem_st.at[3, c])

    def gx_copy(c):
        return pltpu.make_async_copy(go_v.at[cslice(c)], gx_hbm.at[cslice(c)], sem_st.at[4, c])

    def wait_all(mk):
        for c in range(NC):
            mk(c).wait()

    dwe_a[...] = jnp.zeros_like(dwe_a)
    dwo_a[...] = jnp.zeros_like(dwo_a)
    dwin_a[...] = jnp.zeros_like(dwin_a)
    dwout_a[...] = jnp.zeros_like(dwout_a)
    db_a[...] = jnp.zeros_like(db_a)

    ri = jax.lax.broadcasted_iota(jnp.int32, (GR, GR), 0)
    ci = jax.lax.broadcasted_iota(jnp.int32, (GR, GR), 1)
    rd = _idiv(ri, 4)
    rj = ri - rd * 4
    cj = _idiv(ci, DH)
    cd = ci - cj * DH
    hm = rj == cj
    psm = jnp.where(hm & (rd == cd), 1.0, 0.0).astype(BF16)
    hmT = (ci - _idiv(ci, 4) * 4) == _idiv(ri, DH)
    psmT = jnp.where(hmT & (_idiv(ci, 4) == (ri - _idiv(ri, DH) * DH)), 1.0, 0.0).astype(BF16)
    re = jax.lax.broadcasted_iota(jnp.int32, (GR, DH), 0)
    fe = jax.lax.broadcasted_iota(jnp.int32, (GR, DH), 1)
    e_mat = jnp.where(_idiv(re, 4) == fe, 1.0, 0.0).astype(BF16)

    in_cp[1].wait()
    in_cp[2].wait()
    for i in (3, 4, 5, 6):
        in_cp[i].start()
    wqkvT[...] = wqkv_v[...].T
    for g in range(NG):
        rows = slice(g * GR, (g + 1) * GR)
        wph = jnp.concatenate([wphi_v[4 * g + j] for j in range(4)], axis=0)
        bds = jnp.where(hm, _dot_nt(e_mat, wph), 0.0).astype(BF16)
        bds_v[g] = bds
        weT[g * GR:(g + 1) * GR, :] = _dot(bds, wqkvT[g * GR:(g + 1) * GR, :]).astype(BF16)
        weT[D + g * GR:D + (g + 1) * GR, :] = _dot(
            bds, wqkvT[D + g * GR:D + (g + 1) * GR, :]).astype(BF16)
        weT[2 * D + g * GR:2 * D + (g + 1) * GR, :] = _dot(
            psm, wqkvT[2 * D + g * GR:2 * D + (g + 1) * GR, :]).astype(BF16)

    kr = jax.lax.broadcasted_iota(jnp.int32, (160, 96), 0)
    kc = jax.lax.broadcasted_iota(jnp.int32, (160, 96), 1)
    kvmask = (kr - _idiv(kr, 4) * 4) == (kc - _idiv(kc, 4) * 4)
    const16 = jnp.where(
        jax.lax.broadcasted_iota(jnp.int32, (16, C), 0) < 8, 1.0, 0.0).astype(BF16)
    zeros8 = jnp.zeros((8, C), F32)

    def cat_rows(ref, cl, r0, r1):
        parts = [ref[c, r0:r1, :] for c in cl]
        return parts[0] if len(parts) == 1 else jnp.concatenate(parts, axis=1)

    def put_rows(ref, cl, r0, r1, val):
        for k, c in enumerate(cl):
            ref[c, r0:r1, :] = val[:, k * C:(k + 1) * C]

    def wide(cl):
        c0 = cl[0]
        n = len(cl) * C
        if isinstance(c0, int):
            return pl.ds(c0 * C, n)
        return pl.ds(pl.multiple_of(c0 * C, C), n)

    def a_ln(cl, layer):
        h, r = _ln(xs[:, wide(cl)])
        put_rows(actA, cl, A_H, A_H + D, h.astype(BF16))
        for k, c in enumerate(cl):
            rA_v[layer, c] = r[:, k * C:(k + 1) * C]

    def a_fwd1(cl):
        n = len(cl) * C
        work[:, 0:n] = _dot(weT[...], cat_rows(actA, cl, A_H, A_H + D))
        for g in range(NG):
            qp, qn = _phi(work[g * GR:(g + 1) * GR, 0:n])
            put_rows(actA, cl, A_PQ + g * 160, A_PQ + g * 160 + GR, qp.astype(BF16))
            put_rows(actA, cl, A_PQ + g * 160 + GR, A_PQ + (g + 1) * 160, qn.astype(BF16))
            kp, kn = _phi(work[D + g * GR:D + (g + 1) * GR, 0:n])
            put_rows(actA, cl, A_PK + g * 160, A_PK + g * 160 + GR, kp.astype(BF16))
            put_rows(actA, cl, A_PK + g * 160 + GR, A_PK + (g + 1) * 160, kn.astype(BF16))
            put_rows(actA, cl, A_VA + g * 96, A_VA + g * 96 + GR,
                     work[2 * D + g * GR:2 * D + (g + 1) * GR, 0:n].astype(BF16))
            for c in cl:
                actA[c, A_VA + g * 96 + GR:A_VA + (g + 1) * 96, :] = const16

    def kv_dots(cl):
        for g in range(NG):
            kvacc[g] += _dot_nt(cat_rows(actA, cl, A_PK + g * 160, A_PK + (g + 1) * 160),
                                cat_rows(actA, cl, A_VA + g * 96, A_VA + (g + 1) * 96))

    def finish_kv(dst, dstT):
        for g in range(NG):
            kvb = jnp.where(kvmask, kvacc[g], 0.0).astype(BF16)
            dst[g] = kvb
            dstT[g] = kvb.T

    def a_fwd2a(cl, layer):
        for g in range(NG):
            phq = cat_rows(actA, cl, A_PQ + g * 160, A_PQ + (g + 1) * 160)
            na = _dot(kvT_v[layer, g], phq)
            den = na[GR:GR + 8, :] + 1e-6
            put_rows(den_v.at[layer], cl, g * 8, (g + 1) * 8, den)
            o = _g2(_g3(na[0:GR, :]) * (1.0 / den)[None])
            put_rows(actA, cl, A_O + g * GR, A_O + (g + 1) * GR, o.astype(BF16))

    def a_fwd2b(cl):
        xs[:, wide(cl)] += _dot(woPT[...], cat_rows(actA, cl, A_O, A_O + D))

    def b_fwd1(cl, layer):
        n = len(cl) * C
        h, r = _ln(xs[:, wide(cl)])
        hb = h.astype(BF16)
        put_rows(actB, cl, B_H, B_H + D, hb)
        work[0:F, 0:n] = _dot(winT[...], hb)
        z1, gp1 = _gelu_and_grad(work[0:FH, 0:n])
        put_rows(actB, cl, B_Z1, B_Z1 + FH, z1.astype(BF16))
        put_rows(actB, cl, B_GP, B_GP + FH, gp1.astype(BF16))
        zz, gp2 = _gelu_and_grad(work[FH:F, 0:n])
        put_rows(actB, cl, B_GP + FH, B_GP + F, gp2.astype(BF16))
        z2, r2 = _ln(zz)
        z2_v[layer, :, wide(cl)] = z2.astype(BF16)
        for k, c in enumerate(cl):
            rB_v[layer, c] = r[:, k * C:(k + 1) * C]
            r2_v[layer, c] = r2[:, k * C:(k + 1) * C]

    def b_fwd2(c, layer):
        cs = cslice(c)
        gt = _dot_nt(z2_v[layer], wsp_v[cs, :]) + bsp_v[:, cs].astype(F32)
        actB[c, B_G:B_G + FH, :] = gt.astype(BF16)
        u = (actB[c, B_Z1:B_Z1 + FH, :].astype(F32) * gt).astype(BF16)
        xs[:, cs] += _dot(woutT[...], u)

    def b_bwd1(c, layer, first):
        cs = cslice(c)
        dxb = xs[:, cs].astype(BF16)
        du = _dot(wout_v[...], dxb)
        z1 = actB[c, B_Z1:B_Z1 + FH, :].astype(F32)
        gt = actB[c, B_G:B_G + FH, :].astype(F32)
        dwout_a[...] += _dot_nt((z1 * gt).astype(BF16), dxb)
        dg = du * z1
        dz1_v[c] = (du * gt).astype(BF16)
        db_a[:, cs] += jnp.sum(dg, axis=0, keepdims=True)
        dgb = dg.astype(BF16)
        dg_v[:, cs] = dgb
        part = _dot_tn(dgb, z2_v[layer])
        if first:
            dwsp_v[cs, :] = part.astype(BF16)
        else:
            dwsp_v[cs, :] = (dwsp_v[cs, :].astype(F32) + part).astype(BF16)

    def b_bwd2(c, layer):
        cs = cslice(c)
        hb = actB[c, B_H:B_H + D, :]
        dz2 = _dot(dg_v[...], wsp_v[:, cs])
        da1 = (dz1_v[c].astype(F32) * actB[c, B_GP:B_GP + FH, :].astype(F32)).astype(BF16)
        dh1 = _dot(win_v[:, 0:FH], da1)
        dwin_a[:, 0:FH] += _dot_nt(hb, da1)
        dzz = _ln_bwd(dz2, z2_v[layer, :, cs].astype(F32), r2_v[layer, c])
        da2 = (dzz * actB[c, B_GP + FH:B_GP + F, :].astype(F32)).astype(BF16)
        dh = dh1 + _dot(win_v[:, FH:F], da2)
        dwin_a[:, FH:F] += _dot_nt(hb, da2)
        xs[:, cs] += _ln_bwd(dh, hb.astype(F32), rB_v[layer, c])

    def a_bwd1(c, layer):
        cs = cslice(c)
        dxb = xs[:, cs].astype(BF16)
        work[0:D, 0:C] = _dot(woP[...], dxb)
        dwo_a[...] += _dot_nt(actA[c, A_O:A_O + D, :], dxb)
        for g in range(NG):
            do3 = _g3(work[g * GR:(g + 1) * GR, 0:C])
            o3 = _g3(actA[c, A_O + g * GR:A_O + (g + 1) * GR, :].astype(F32))
            rden = 1.0 / den_v[layer, c, g * 8:(g + 1) * 8, :]
            dnum = _g2(do3 * rden[None])
            dden = (-0.5) * _red_sum(do3 * o3) * rden
            dna = jnp.concatenate([dnum, dden, zeros8], axis=0).astype(BF16)
            phq = actA[c, A_PQ + g * 160:A_PQ + (g + 1) * 160, :]
            dphq = _dot(kv_v[layer, g], dna)
            kvacc[g] += _dot_nt(phq, dna)
            phqf = phq.astype(F32)
            dpq = _phi_bwd(phqf[0:GR], phqf[GR:160], dphq[0:GR], dphq[GR:160])
            dpq_v[c, g * GR:(g + 1) * GR, :] = dpq.astype(BF16)

    def a_bwd2(c, layer):
        cs = cslice(c)
        dqkv_v[0:D, :] = dpq_v[c]
        for g in range(NG):
            va = actA[c, A_VA + g * 96:A_VA + (g + 1) * 96, :]
            phk = actA[c, A_PK + g * 160:A_PK + (g + 1) * 160, :]
            dphk = _dot(dkv_v[g], va)
            dv = _dot(dkvT_v[g, 0:GR, :], phk)
            phkf = phk.astype(F32)
            dpk = _phi_bwd(phkf[0:GR], phkf[GR:160], dphk[0:GR], dphk[GR:160])
            dqkv_v[D + g * GR:D + (g + 1) * GR, :] = dpk.astype(BF16)
            dqkv_v[2 * D + g * GR:2 * D + (g + 1) * GR, :] = dv.astype(BF16)
        dqkv = dqkv_v[...]
        hb = actA[c, A_H:A_H + D, :]
        dh = _dot(we[...], dqkv)
        dwe_a[...] += _dot_nt(dqkv, hb)
        xs[:, cs] += _ln_bwd(dh, hb.astype(F32), rA_v[layer, c])

    def chunk_loop(body):
        def wrapped(c, carry):
            body(c)
            return carry
        jax.lax.fori_loop(0, NC, wrapped, 0)

    def zero_kvacc():
        kvacc[...] = jnp.zeros_like(kvacc)

    in_cp[0].wait()
    in_cp[7].start()
    zero_kvacc()

    NP = NC // 2

    def pair(i):
        return [2 * i, 2 * i + 1]

    def p1x(i):
        w = wide(pair(i))
        xs[:, w] = x_v[w, :].T.astype(F32)
        a_ln(pair(i), 0)

    with jax.named_scope("p1"):
        p1x(0)

        def p1_body(i, carry):
            a_fwd1(pair(i))
            p1x(i + 1)
            kv_dots(pair(i))
            return carry
        jax.lax.fori_loop(0, NP - 1, p1_body, 0)
        for i in (3, 4, 5, 6):
            in_cp[i].wait()
        a_fwd1(pair(NP - 1))
        winT[...] = win_v[...].T
        woutT[...] = wout_v[...].T
        for g in range(NG):
            woP[g * GR:(g + 1) * GR, :] = _dot(psm, wo_v[g * GR:(g + 1) * GR, :]).astype(BF16)
        woPT[...] = woP[...].T
        kv_dots(pair(NP - 1))
    finish_kv(kv_v.at[0], kvT_v.at[0])

    def p24(layer):
        a_fwd2a(pair(0), layer)
        a_fwd2b(pair(0))
        if layer == 0:
            stash_out_A(0).start()
            stash_out_A(1).start()
        else:
            we[:, 1536:1920] = weT[1536:1920, :].T

        def body(i, carry):
            if layer == 1:
                stash_out_B(2 * i).wait()
                stash_out_B(2 * i + 1).wait()
            a_fwd2a(pair(i + 1), layer)
            b_fwd1(pair(i), layer)
            a_fwd2b(pair(i + 1))
            if layer == 0:
                stash_out_A(2 * i + 2).start()
                stash_out_A(2 * i + 3).start()
            else:
                o1 = pl.multiple_of(i * 512, 512)
                we[:, pl.ds(o1, 512)] = weT[pl.ds(o1, 512), :].T
            return carry
        jax.lax.fori_loop(0, NP - 1, body, 0)
        if layer == 1:
            stash_out_B(NC - 2).wait()
            stash_out_B(NC - 1).wait()
        b_fwd1(pair(NP - 1), layer)

    with jax.named_scope("p2"):
        p24(0)

    in_cp[7].wait()
    in_cp[8].start()
    zero_kvacc()

    def p3x(c):
        b_fwd2(c, 0)
        stash_out_B(c).start()
        a_ln([c], 1)

    with jax.named_scope("p3"):
        stash_out_A(0).wait()
        p3x(0)

        def p3_body(c, carry):
            stash_out_A(c + 1).wait()
            a_fwd1([c])
            p3x(c + 1)
            kv_dots([c])
            return carry
        jax.lax.fori_loop(0, NC - 1, p3_body, 0)
        a_fwd1([NC - 1])
        kv_dots([NC - 1])
    finish_kv(kv_v.at[1], kvT_v.at[1])

    with jax.named_scope("p4"):
        p24(1)

    in_cp[8].wait()

    def p5x(c):
        b_fwd2(c, 1)

    def p5y(c):
        cs = cslice(c)
        x_v[cs, :] = xs[:, cs].T.astype(BF16)
        xs[:, cs] = go_v[cs, :].T.astype(F32)
        b_bwd1(c, 1, True)
    def p5(c):
        p5x(c)
        p5y(c)
    chunk_loop(p5)
    out_cp = pltpu.make_async_copy(x_v, out_hbm, sem_out.at[0])
    out_cp.start()
    zero_kvacc()

    def p6x(c):
        b_bwd2(c, 1)
        stash_in_B(c).start()

    def p6y(c):
        a_bwd1(c, 1)
    def p6(c):
        p6x(c)
        p6y(c)
    chunk_loop(p6)
    finish_kv(dkv_v, dkvT_v)

    def p7x(c):
        stash_in_B(c).wait()
        a_bwd2(c, 1)
        stash_in_A(c).start()

    def p7y(c):
        b_bwd1(c, 0, False)
    def p7(c):
        p7x(c)
        p7y(c)
    chunk_loop(p7)
    dwsp_cp = pltpu.make_async_copy(dwsp_v, dwsp_hbm, sem_out.at[1])
    dwsp_cp.start()
    db_v[...] = db_a[...].astype(BF16)
    db_cp = pltpu.make_async_copy(db_v, db_hbm, sem_out.at[2])
    db_cp.start()
    wout_v[...] = dwout_a[...].astype(BF16)
    dwout_cp = pltpu.make_async_copy(wout_v, dwout_hbm, sem_out.at[3])
    dwout_cp.start()
    zero_kvacc()

    def p8x(c):
        stash_in_A(c).wait()
        b_bwd2(c, 0)

    def p8y(c):
        a_bwd1(c, 0)
    def p8(c):
        p8x(c)
        p8y(c)
    chunk_loop(p8)
    finish_kv(dkv_v, dkvT_v)
    win_v[...] = dwin_a[...].astype(BF16)
    dwin_cp = pltpu.make_async_copy(win_v, dwin_hbm, sem_out.at[4])
    dwin_cp.start()
    for g in range(NG):
        wo_v[g * GR:(g + 1) * GR, :] = _dot(
            psmT, dwo_a[g * GR:(g + 1) * GR, :].astype(BF16)).astype(BF16)
    dwo_cp = pltpu.make_async_copy(wo_v, dwo_hbm, sem_out.at[5])
    dwo_cp.start()

    def p9(c):
        cs = cslice(c)
        a_bwd2(c, 0)
        go_v[cs, :] = xs[:, cs].T.astype(BF16)
        gx_copy(c).start()
    chunk_loop(p9)

    dwqkv_cps = []
    for part in range(3):
        for g in range(NG):
            rows = slice(part * D + g * GR, part * D + (g + 1) * GR)
            dpart = dwe_a[rows, :].astype(BF16)
            mat = psmT if part == 2 else bds_v[g].T
            weT[rows, :] = _dot(mat, dpart).astype(BF16)
        wqkv_v[:, part * D:(part + 1) * D] = weT[part * D:(part + 1) * D, :].T
        cp = pltpu.make_async_copy(
            wqkv_v.at[:, part * D:(part + 1) * D], dwqkv_hbm.at[:, part * D:(part + 1) * D],
            sem_out.at[6 + part])
        cp.start()
        dwqkv_cps.append(cp)
    for g in range(NG):
        dq = dwe_a[g * GR:(g + 1) * GR, :].astype(BF16)
        dk = dwe_a[D + g * GR:D + (g + 1) * GR, :].astype(BF16)
        m = (_dot_nt(wqkvT[g * GR:(g + 1) * GR, :], dq)
             + _dot_nt(wqkvT[D + g * GR:D + (g + 1) * GR, :], dk))
        m = jnp.where(hmT, m, 0.0)
        dwp = jnp.dot(m, e_mat.astype(F32), preferred_element_type=F32,
                      precision=jax.lax.Precision.HIGHEST).astype(BF16)
        for j in range(4):
            dwphi_v[4 * g + j] = dwp[j * DH:(j + 1) * DH, :]
    dwphi_cp = pltpu.make_async_copy(dwphi_v, dwphi_hbm, sem_out.at[9])
    dwphi_cp.start()

    for cp in (out_cp, dwsp_cp, db_cp, dwout_cp, dwin_cp, dwo_cp, dwphi_cp, *dwqkv_cps):
        cp.wait()
    wait_all(gx_copy)


@jax.jit
def pallas_interleave_layers__linear_kernel_hedgehog__mixer_gmlp__prompt_kernel(
    A_x: jax.Array,
    A_wqkv: jax.Array,
    A_w_phi: jax.Array,
    A_wo: jax.Array,
    B_x: jax.Array,
    B_w_in: jax.Array,
    B_w_sp: jax.Array,
    B_b_sp: jax.Array,
    B_w_out: jax.Array,
    grad_out: jax.Array,
):
    del B_x
    x2 = A_x.reshape(S, D)
    go2 = grad_out.reshape(S, D)
    bsp2 = B_b_sp.reshape(1, S)

    sds = jax.ShapeDtypeStruct
    out_shape = (
        sds((S, D), BF16),
        sds((S, D), BF16),
        sds((D, 3 * D), BF16),
        sds((32, DH, DH), BF16),
        sds((D, D), BF16),
        sds((D, F), BF16),
        sds((S, S), BF16),
        sds((1, S), BF16),
        sds((FH, D), BF16),
        sds((NC, A_ROWS, C), BF16),
        sds((NC, B_ROWS, C), BF16),
    )
    V = pltpu.VMEM
    scratch = [
        V((S, D), BF16), V((S, D), BF16), V((D, 3 * D), BF16), V((32, DH, DH), BF16),
        V((D, D), BF16), V((D, F), BF16), V((S, S), BF16), V((1, S), BF16), V((FH, D), BF16),
        V((3 * D, D), BF16), V((D, 3 * D), BF16), V((D, D), BF16), V((D, D), BF16),
        V((F, D), BF16), V((D, FH), BF16), V((NG, GR, GR), BF16), V((3 * D, D), BF16),
        V((D, S), F32), V((NC, A_ROWS, C), BF16), V((NC, B_ROWS, C), BF16),
        V((2, FH, S), BF16), V((2, NC, 64, C), F32),
        V((2, NC, 1, C), F32), V((2, NC, 1, C), F32), V((2, NC, 1, C), F32),
        V((NG, 160, 96), F32), V((2, NG, 160, 96), BF16), V((2, NG, 96, 160), BF16),
        V((NG, 160, 96), BF16), V((NG, 96, 160), BF16),
        V((FH, S), BF16), V((NC, FH, C), BF16), V((NC, D, C), BF16),
        V((3 * D, 2 * C), F32), V((3 * D, C), BF16),
        V((3 * D, D), F32), V((D, D), F32), V((D, F), F32), V((FH, D), F32),
        V((1, S), F32), V((S, S), BF16), V((32, DH, DH), BF16), V((1, S), BF16),
        pltpu.SemaphoreType.DMA((9,)), pltpu.SemaphoreType.DMA((10,)),
        pltpu.SemaphoreType.DMA((5, NC)),
    ]
    any_spec = pl.BlockSpec(memory_space=pl.ANY)
    res = pl.pallas_call(
        _kernel,
        out_shape=out_shape,
        in_specs=[any_spec] * 9,
        out_specs=tuple([any_spec] * len(out_shape)),
        scratch_shapes=scratch,
        compiler_params=pltpu.CompilerParams(vmem_limit_bytes=125 * 1024 * 1024),
    )(x2, A_wqkv, A_w_phi, A_wo, B_w_in, B_w_sp, bsp2, B_w_out, go2)
    out, gx, dwqkv, dwphi, dwo, dwin, dwsp, db, dwout = res[:9]
    return (
        out.reshape(1, S, D),
        gx.reshape(1, S, D),
        dwqkv,
        dwphi,
        dwo,
        dwin,
        dwsp,
        db.reshape(S),
        dwout,
    )
```
